```python
import jax
import jax.numpy as jnp

def _softmax(x, axis=-1):
    return jax.nn.softmax(x, axis=axis)

def _gelu(x):
    return jax.nn.gelu(x, approximate=True)

def _silu(x):
    return jax.nn.silu(x)

def _sigmoid(x):
    return jax.nn.sigmoid(x)

def _layernorm(x, axis=-1, eps=1e-05):
    m = jnp.mean(x, axis=axis, keepdims=True)
    v = jnp.var(x, axis=axis, keepdims=True)
    return (x - m) / jnp.sqrt(v + eps)

def _scatter_add(tgt, idx, src, axis=0):
    return tgt.at[idx].add(src)

def _segment_sum(src, seg, n):
    return jax.ops.segment_sum(src, seg, n)

class _Rng:

    def __init__(self, key):
        self._k = key

    def _next(self):
        self._k, sub = jax.random.split(self._k)
        return sub

    def normal(self, shape):
        return jax.random.normal(self._next(), shape, dtype=jnp.bfloat16)

    def randint(self, lo, hi, shape):
        return jax.random.randint(self._next(), shape, lo, hi, dtype=jnp.int32)

    def uniform(self, shape, lo=0.0, hi=1.0):
        return jax.random.uniform(self._next(), shape, jnp.bfloat16, lo, hi)

    def permutation(self, n):
        return jax.random.permutation(self._next(), n)
kernel_name = 'concat_heads__memory_aug_recurrent_mem_tr__sliding_local_dilated__prompt'

def setup_inputs():
    _rng = _Rng(jax.random.key(int.from_bytes(__import__("os").urandom(4), "little")))
    _w = lambda a: (lambda t: t.astype(jnp.bfloat16) if jnp.issubdtype(t.dtype, jnp.floating) else t)(jnp.asarray(a))

    def _A_setup():
        B, S, Dm = (1, 2048, 1024)
        H, Dh = (32, 128)
        M, seg = (8, 32)
        seg = min(seg, S)
        S = S // seg * seg
        return {'x': _w((lambda *s: _rng.normal(s) * 0.05)(B, S, Dm)), 'mem0': _w((lambda *s: _rng.normal(s) * 0.05)(B, M, Dm)), 'Wq': _w((lambda *s: _rng.normal(s) * 0.05)(Dm, H, Dh) * Dm ** (-0.5)), 'Wk': _w((lambda *s: _rng.normal(s) * 0.05)(Dm, H, Dh) * Dm ** (-0.5)), 'Wv': _w((lambda *s: _rng.normal(s) * 0.05)(Dm, H, Dh) * Dm ** (-0.5)), 'Wo': _w((lambda *s: _rng.normal(s) * 0.05)(H, Dh, Dm) * (H * Dh) ** (-0.5)), 'seg_len': seg}
    _A_in = _A_setup()

    def _B_setup():
        B, S, D = (1, 2048, 1024)
        return {'x': _w((lambda *s: _rng.normal(s) * 0.05)(B, S, D)), 'wqkv': _w((lambda *s: _rng.normal(s) * 0.05)(D, 3 * D)), 'wo': _w((lambda *s: _rng.normal(s) * 0.05)(D, D))}
    _B_in = _B_setup()
    return {'A_x': _A_in['x'], 'A_mem0': _A_in['mem0'], 'A_Wq': _A_in['Wq'], 'A_Wk': _A_in['Wk'], 'A_Wv': _A_in['Wv'], 'A_Wo': _A_in['Wo'], 'A_seg_len': _A_in['seg_len'], 'B_x': _B_in['x'], 'B_wqkv': _B_in['wqkv'], 'B_wo': _B_in['wo']}

def reference(A_x, A_mem0, A_Wq, A_Wk, A_Wv, A_Wo, A_seg_len, B_x, B_wqkv, B_wo):

    def _A_ref(x, mem0, Wq, Wk, Wv, Wo, seg_len):
        B, S, Dm = x.shape
        H, Dh = (Wq.shape[1], Wq.shape[2])
        M = mem0.shape[1]
        scale = Dh ** (-0.5)
        n_seg = S // seg_len
        L = M + seg_len
        idx = jnp.arange(L)
        mask = (idx[:, None] < M) | (idx[:, None] >= idx[None, :])
        mem = mem0
        outs = []
        for s in range(n_seg):
            xs = x[:, s * seg_len:(s + 1) * seg_len, :].copy()
            h = jnp.concatenate([mem, xs], axis=1)
            q = jnp.einsum('btd,dhe->bhte', h, Wq)
            k = jnp.einsum('btd,dhe->bhte', h, Wk)
            v = jnp.einsum('btd,dhe->bhte', h, Wv)
            scores = jnp.einsum('bhqe,bhke->bhqk', q, k) * scale
            scores = jnp.where(mask[None, None], scores, -1000000000.0)
            p = _softmax(scores, axis=-1)
            o = jnp.einsum('bhqk,bhke->bhqe', p, v)
            o = jnp.einsum('bhte,hed->btd', o, Wo)
            mem = o[:, :M, :].copy()
            outs.append(o[:, M:, :])
        return jnp.concatenate(outs, axis=1)

    def _B_ref(x, wqkv, wo):
        B, S, D = x.shape
        H = 32
        Dh = D // H
        W, dil = (8, 2)
        qkv = (lambda x, *d: x.transpose(*d))((x @ wqkv).reshape(B, S, 3, H, Dh), 2, 0, 3, 1, 4)
        q, k, v = (qkv[0], qkv[1], qkv[2])
        scale = Dh ** (-0.5)
        pos = jnp.arange(S)
        off = jnp.arange(W) * dil
        idx = pos[:, None] - off[None, :]
        mask = idx >= 0
        idx_c = jnp.where(mask, idx, 0).reshape(-1)
        kg = k[:, :, idx_c, :].reshape(B, H, S, W, Dh)
        vg = v[:, :, idx_c, :].reshape(B, H, S, W, Dh)
        logits = jnp.einsum('bhsd,bhswd->bhsw', q, kg) * scale
        logits = jnp.where(mask[None, None, :, :], logits, -1000000000.0)
        attn = _softmax(logits, axis=-1)
        o = jnp.einsum('bhsw,bhswd->bhsd', attn, vg)
        return (lambda x, *d: x.transpose(*d))(o, 0, 2, 1, 3).reshape(B, S, D) @ wo
    a = _A_ref(A_x, A_mem0, A_Wq, A_Wk, A_Wv, A_Wo, A_seg_len)
    b = _B_ref(B_x, B_wqkv, B_wo)
    return jnp.concatenate([a, b], axis=-1)
```

```python
import functools

import jax
import jax.numpy as jnp
from jax import lax
from jax.experimental import pallas as pl
from jax.experimental.pallas import tpu as pltpu

F32 = jnp.float32
BF16 = jnp.bfloat16
I32 = jnp.int32

LANES = 128
NEG = -1000000000.0

B_HEADS = 32
B_WIN = 8
B_DIL = 2
HALO = 16
SUB = 128
NSUB = 2
GRP = 16

LAG_S = 1
LAG_P = 2


def _as_bf16(words):
    return pltpu.bitcast(words, BF16)


def _kernel(
    xa_hbm, mem_hbm, wq_hbm, wk_hbm, wv_hbm, woa_hbm, xb_hbm, wb_hbm, wob_hbm,
    out_hbm,
    wa, woa, xa, mem0, outa, hbuf, obuf,
    xb, wb, wob_raw, wob, outb,
    q0, q1, k0, k1, v0, v1, ob0, ob1,
    sem_b, sem_wa, sem_misc, sem_out,
    *, seq, dm, heads, n_mem, seg,
):
    kt = dm // LANES
    n_iter = seq // (SUB * NSUB)
    regions = dm // 16
    reg_per_iter = regions // n_iter
    reg_rows = 16 * heads // 2
    wa_flat = wa.reshape(3 * regions * reg_rows, LANES)
    wa_reg = wa.reshape(3 * regions, reg_rows, LANES)

    def col_copies(src_hbm, dst, sem):
        src = src_hbm.bitcast(I32)
        return [
            pltpu.make_async_copy(src.at[:, pl.ds(j * LANES, LANES)], dst.at[j], sem)
            for j in range(dst.shape[0])
        ]

    def wa_copies(i):
        rows = reg_per_iter * reg_rows
        return [
            pltpu.make_async_copy(
                w.bitcast(I32).at[pl.ds(i * rows, rows)],
                wa_flat.at[pl.ds(m * regions * reg_rows + i * rows, rows)],
                sem_wa.at[i],
            )
            for m, w in enumerate((wq_hbm, wk_hbm, wv_hbm))
        ]

    wb_cp = col_copies(wb_hbm, wb, sem_b.at[0])
    xb_cp = col_copies(xb_hbm, xb, sem_b.at[1])
    wob_cp = col_copies(wob_hbm, wob_raw, sem_b.at[2])
    woa_cp = col_copies(woa_hbm, woa, sem_misc.at[0])
    xa_cp = pltpu.make_async_copy(xa_hbm, xa, sem_misc.at[1])
    mem_cp = pltpu.make_async_copy(mem_hbm, mem0, sem_misc.at[2])

    def outb_copy(i):
        rows = SUB * NSUB
        r0 = pl.multiple_of(i * rows, rows)
        return pltpu.make_async_copy(
            outb.at[pl.ds(r0, rows)], out_hbm.at[pl.ds(r0, rows), pl.ds(dm, dm)], sem_out.at[0]
        )

    def outa_copy(t):
        r0 = pl.multiple_of(t * seg, seg)
        return pltpu.make_async_copy(
            outa.at[pl.ds(r0, seg)], out_hbm.at[pl.ds(r0, seg), pl.ds(0, dm)], sem_out.at[1]
        )

    for cp in wb_cp + xb_cp + wob_cp:
        cp.start()
    for cp in wb_cp:
        cp.wait()
    for i in range(n_iter):
        for cp in wa_copies(i):
            cp.start()
    for cp in woa_cp + [xa_cp, mem_cp]:
        cp.start()

    lane = lax.broadcasted_iota(I32, (8, LANES), 1)

    def permute_wb(r, carry):
        r0 = pl.multiple_of(r * 8, 8)
        for m in range(3):
            x = [wb[m * kt + a, pl.ds(r0, 8), :] for a in range(kt)]
            for bit in range(3):
                s = 1 << bit
                low = (lane & (4 * s)) == 0
                y = list(x)
                for a in range(kt):
                    if a & s == 0:
                        y[a] = jnp.where(low, x[a], pltpu.roll(x[a + s], 4 * s, 1))
                        y[a + s] = jnp.where(low, pltpu.roll(x[a], LANES - 4 * s, 1), x[a + s])
                x = y
            for a in range(kt):
                wb[m * kt + a, pl.ds(r0, 8), :] = x[a]
        return carry

    lax.fori_loop(0, dm // 16, permute_wb, None)

    for cp in wob_cp:
        cp.wait()

    def permute_wob(n, carry):
        for t in range(kt):
            for g in range(4):
                for b in range(2):
                    rows = wob_raw[n, pl.ds(g * 16 + t * 2 + b, 8, stride=64), :]
                    wob[n, pl.ds(t * 64 + g * 16 + b, 8, stride=2), :] = rows
        return carry

    lax.fori_loop(0, kt, permute_wob, None)

    zeros_halo = jnp.zeros((kt, HALO, LANES), F32)
    k1[:, SUB:SUB + HALO, :] = zeros_halo
    v1[:, SUB:SUB + HALO, :] = zeros_halo

    for cp in xb_cp:
        cp.wait()

    b_scale = float((dm // B_HEADS) ** -0.5)
    lane_g = lax.broadcasted_iota(I32, (GRP, LANES), 1)
    row_g = lax.broadcasted_iota(I32, (GRP, LANES), 0)
    even1 = (lane_g & 1) == 0
    even2 = (lane_g & 2) == 0

    def b_project(row0, q_s, k_s, v_s):
        w0 = pl.multiple_of(row0 // 2, SUB // 2)
        x = jnp.concatenate(
            [_as_bf16(xb[j, pl.ds(w0, SUB // 2), :]) for j in range(kt)], axis=1
        )
        for m, (dst, off) in enumerate(((q_s, 0), (k_s, HALO), (v_s, HALO))):
            for t in range(kt):
                y = jnp.dot(x, _as_bf16(wb[m * kt + t]), preferred_element_type=F32)
                dst[t, off:off + SUB, :] = y

    def b_attend(row0, q_s, k_s, v_s, o_s, first):
        for g in range(SUB // GRP):
            base = HALO + g * GRP
            logits = []
            for w in range(B_WIN):
                acc = None
                for t in range(kt):
                    term = q_s[t, g * GRP:(g + 1) * GRP, :] * k_s[t, pl.ds(base - B_DIL * w, GRP), :]
                    acc = term if acc is None else acc + term
                acc = acc + jnp.where(even1, pltpu.roll(acc, LANES - 1, 1), pltpu.roll(acc, 1, 1))
                acc = acc + jnp.where(even2, pltpu.roll(acc, LANES - 2, 1), pltpu.roll(acc, 2, 1))
                acc = acc * b_scale
                if first and g * GRP < B_DIL * w:
                    acc = jnp.where(row0 + g * GRP + row_g >= B_DIL * w, acc, NEG)
                logits.append(acc)
            top = functools.reduce(jnp.maximum, logits)
            e = [jnp.exp(l - top) for l in logits]
            inv = 1.0 / functools.reduce(lambda a, b: a + b, e)
            p = [x * inv for x in e]
            for t in range(kt):
                acc = None
                for w in range(B_WIN):
                    term = p[w] * v_s[t, pl.ds(base - B_DIL * w, GRP), :]
                    acc = term if acc is None else acc + term
                o_s[t, g * GRP // 2:(g + 1) * GRP // 2, :] = pltpu.bitcast(acc.astype(BF16), I32)

    def b_output(row0, o_s):
        o = jnp.concatenate([_as_bf16(o_s[t]) for t in range(kt)], axis=1)
        for n in range(kt):
            y = jnp.dot(o, _as_bf16(wob[n]), preferred_element_type=F32)
            outb[pl.ds(row0, SUB), n * LANES:(n + 1) * LANES] = y.astype(BF16)

    def relayout_wa(i):
        half = heads // 2
        for m in range(3):
            for r in range(reg_per_iter):
                reg = m * regions + i * reg_per_iter + r
                src = [wa_reg[reg, pl.ds(8 * u, 8), :] for u in range(reg_rows // 8)]
                per_d = half // 8
                for pair in range(8):
                    for part in range(per_d):
                        a = src[(2 * pair) * per_d + part]
                        b = src[(2 * pair + 1) * per_d + part]
                        lo = (a & 0xFFFF) | (b << 16)
                        hi = lax.shift_right_logical(a, 16) | (b & -65536)
                        wa_reg[reg, pl.ds(part * 64 + pair, 8, stride=8), :] = lo
                        wa_reg[reg, pl.ds(half * 8 + part * 64 + pair, 8, stride=8), :] = hi

    def b_step(i, carry):
        for cp in wa_copies(i):
            cp.wait()
        row_a = pl.multiple_of(i * (SUB * NSUB), SUB * NSUB)
        row_b = pl.multiple_of(row_a + SUB, SUB)
        k0[:, 0:HALO, :] = k1[:, SUB:SUB + HALO, :]
        v_prev = v1[:, SUB:SUB + HALO, :]
        b_project(row_a, q0, k0, v0)
        v_first = jnp.broadcast_to(v0[:, HALO:HALO + 1, :], (kt, HALO, LANES))
        v0[:, 0:HALO, :] = jnp.where(i == 0, v_first, v_prev)
        k1[:, 0:HALO, :] = k0[:, SUB:SUB + HALO, :]
        v1[:, 0:HALO, :] = v0[:, SUB:SUB + HALO, :]
        b_project(row_b, q1, k1, v1)
        b_attend(row_a, q0, k0, v0, ob0, True)
        b_output(row_a, ob0)
        b_attend(row_b, q1, k1, v1, ob1, False)
        b_output(row_b, ob1)
        relayout_wa(i)
        outb_copy(i).start()
        return carry

    lax.fori_loop(0, n_iter, b_step, None)

    for cp in woa_cp + [xa_cp, mem_cp]:
        cp.wait()

    rows = n_mem + seg
    a_scale = float(LANES ** -0.5)
    hbuf[0:n_mem, :] = mem0[...].astype(F32)
    row = lax.broadcasted_iota(I32, (rows, rows), 0)
    col = lax.broadcasted_iota(I32, (rows, rows), 1)

    def a_step(t, carry):
        r0 = pl.multiple_of(t * seg, seg)
        hbuf[n_mem:rows, :] = xa[pl.ds(r0, seg), :].astype(F32)
        visible = (row < n_mem) | (row >= col)
        qkv, prob = {}, {}

        def project(h):
            slot = (h % 2) * (heads // 2) + h // 2
            w = jnp.concatenate(
                [
                    _as_bf16(wa[pl.ds(m * regions, regions), slot].reshape(dm // 2, LANES))
                    for m in range(3)
                ],
                axis=1,
            )
            qkv[h] = jnp.dot(hbuf[...], w, preferred_element_type=F32)

        def scores(h):
            q = qkv[h][:, 0:LANES]
            k = qkv[h][:, LANES:2 * LANES].astype(BF16)
            s = lax.dot_general(q, k, (((1,), (1,)), ((), ())), preferred_element_type=F32)
            s = jnp.where(visible, s * a_scale, NEG)
            e = jnp.exp(s - jnp.max(s, axis=1, keepdims=True))
            prob[h] = e / jnp.sum(e, axis=1, keepdims=True)

        def mix(h):
            v = qkv.pop(h)[:, 2 * LANES:].astype(BF16)
            obuf[:, h * LANES:(h + 1) * LANES] = jnp.dot(
                prob.pop(h), v, preferred_element_type=F32
            )

        for i in range(heads + LAG_P):
            if i < heads:
                project(i)
            if 0 <= i - LAG_S < heads:
                scores(i - LAG_S)
            if 0 <= i - LAG_P < heads:
                mix(i - LAG_P)

        for n in range(kt):
            y = jnp.dot(obuf[...], _as_bf16(woa[n]), preferred_element_type=F32).astype(BF16)
            hbuf[0:n_mem, n * LANES:(n + 1) * LANES] = y[0:n_mem].astype(F32)
            outa[pl.ds(r0, seg), n * LANES:(n + 1) * LANES] = y[n_mem:rows]
        outa_copy(t).start()
        return carry

    n_seg = seq // seg
    lax.fori_loop(0, n_seg, a_step, None)

    pltpu.make_async_copy(outb, out_hbm.at[:, pl.ds(dm, dm)], sem_out.at[0]).wait()
    pltpu.make_async_copy(outa, out_hbm.at[:, pl.ds(0, dm)], sem_out.at[1]).wait()


@functools.partial(jax.jit, static_argnames=("A_seg_len",))
def pallas_concat_heads__memory_aug_recurrent_mem_tr__sliding_local_dilated__prompt_kernel(
    A_x: jax.Array,
    A_mem0: jax.Array,
    A_Wq: jax.Array,
    A_Wk: jax.Array,
    A_Wv: jax.Array,
    A_Wo: jax.Array,
    A_seg_len: int,
    B_x: jax.Array,
    B_wqkv: jax.Array,
    B_wo: jax.Array,
):
    batch, seq, dm = A_x.shape
    _, heads, dh = A_Wq.shape
    n_mem = A_mem0.shape[1]
    seg = int(A_seg_len)
    assert batch == 1 and B_x.shape == (1, seq, dm)
    assert dh == LANES and dm == 8 * LANES and dm // B_HEADS == 32 and heads % 16 == 0
    assert n_mem % 8 == 0 and seg % 16 == 0 and seq % seg == 0 and seq % (SUB * NSUB) == 0
    kt = dm // LANES
    rows = n_mem + seg
    n_iter = seq // (SUB * NSUB)
    assert (dm // 16) % n_iter == 0

    any_spec = pl.BlockSpec(memory_space=pl.ANY)
    scratch = [
        pltpu.VMEM((3 * dm // 16, heads, 8, LANES), I32),
        pltpu.VMEM((kt, heads * dh // 2, LANES), I32),
        pltpu.VMEM((seq, dm), BF16),
        pltpu.VMEM((n_mem, dm), BF16),
        pltpu.VMEM((seq, dm), BF16),
        pltpu.VMEM((rows, dm), F32),
        pltpu.VMEM((rows, heads * dh), F32),
        pltpu.VMEM((kt, seq // 2, LANES), I32),
        pltpu.VMEM((3 * kt, dm // 2, LANES), I32),
        pltpu.VMEM((kt, dm // 2, LANES), I32),
        pltpu.VMEM((kt, dm // 2, LANES), I32),
        pltpu.VMEM((seq, dm), BF16),
        pltpu.VMEM((kt, SUB, LANES), F32),
        pltpu.VMEM((kt, SUB, LANES), F32),
        pltpu.VMEM((kt, HALO + SUB, LANES), F32),
        pltpu.VMEM((kt, HALO + SUB, LANES), F32),
        pltpu.VMEM((kt, HALO + SUB, LANES), F32),
        pltpu.VMEM((kt, HALO + SUB, LANES), F32),
        pltpu.VMEM((kt, SUB // 2, LANES), I32),
        pltpu.VMEM((kt, SUB // 2, LANES), I32),
        pltpu.SemaphoreType.DMA((3,)),
        pltpu.SemaphoreType.DMA((n_iter,)),
        pltpu.SemaphoreType.DMA((3,)),
        pltpu.SemaphoreType.DMA((2,)),
    ]
    out = pl.pallas_call(
        functools.partial(_kernel, seq=seq, dm=dm, heads=heads, n_mem=n_mem, seg=seg),
        out_shape=jax.ShapeDtypeStruct((seq, 2 * dm), BF16),
        in_specs=[any_spec] * 9,
        out_specs=any_spec,
        scratch_shapes=scratch,
        compiler_params=pltpu.CompilerParams(vmem_limit_bytes=100 * 1024 * 1024),
    )(
        A_x.reshape(seq, dm),
        A_mem0.reshape(n_mem, dm),
        A_Wq.reshape(dm * heads, dh),
        A_Wk.reshape(dm * heads, dh),
        A_Wv.reshape(dm * heads, dh),
        A_Wo.reshape(heads * dh, dm),
        B_x.reshape(seq, dm),
        B_wqkv,
        B_wo,
    )
    return out.reshape(1, seq, 2 * dm)
```

```python
import functools

import jax
import jax.numpy as jnp
from jax import lax
from jax.experimental import pallas as pl
from jax.experimental.pallas import tpu as pltpu

F32 = jnp.float32
BF16 = jnp.bfloat16
I32 = jnp.int32

LANES = 128
NEG = -1000000000.0

B_HEADS = 32
B_WIN = 8
B_DIL = 2

HALO = 16
SUB = 128
CHUNK = 2 * SUB
GRP = 16
WQ_BLOCKS = 2
PERM_LAG = 4
LAG_S = 4
LAG_P = 5
A_UNROLL = 1


def _as_bf16(words):
    return pltpu.bitcast(words, BF16)


def _start(copies):
    for cp in copies:
        cp.start()


def _wait(copies):
    for cp in copies:
        cp.wait()


def _aligned(start, multiple):
    return start if isinstance(start, int) else pl.multiple_of(start, multiple)


def _kernel(
    xa_hbm, mem_hbm, wq_hbm, wk_hbm, wv_hbm, woa_hbm, xb_hbm, wb_hbm, wob_hbm,
    out_hbm,
    wa, woa, xa, mem0, outa, hbuf, obuf, pbuf,
    xb, wb_raw, wb, wob, outb, q_all, k0, k1, v0, v1, p0, p1, ob0, ob1, zero,
    sem_xb, sem_wb, sem_wa, sem_late, sem_out,
    *, seq, dm, heads, n_mem, seg,
):
    kt = dm // LANES
    n_iter = seq // CHUNK
    regions = dm // 16
    reg_per_iter = regions // n_iter
    reg_rows = 16 * heads // 2
    slots = regions + 1
    wa_flat = wa.reshape(3 * slots * reg_rows, LANES)
    wa_reg = wa.reshape(3 * slots, reg_rows, LANES)

    def col_copy(src_hbm, dst, j, r0, n, sem):
        return pltpu.make_async_copy(
            src_hbm.bitcast(I32).at[pl.ds(r0, n), pl.ds(j * LANES, LANES)],
            dst.at[j, pl.ds(r0, n)],
            sem,
        )

    wq_rows = dm // 2 // WQ_BLOCKS
    xb_bounds = (0, CHUNK // 2, seq // 4, seq // 2)

    def wq_copies(u):
        return [col_copy(wb_hbm, wb_raw, j, u * wq_rows, wq_rows, sem_wb.at[u]) for j in range(kt)]

    def wkv_copies():
        return [
            col_copy(wb_hbm, wb_raw, j, 0, dm // 2, sem_wb.at[WQ_BLOCKS]) for j in range(kt, 3 * kt)
        ]

    def xb_copies(u):
        r0, r1 = xb_bounds[u:u + 2]
        return [col_copy(xb_hbm, xb, j, r0, r1 - r0, sem_xb.at[u]) for j in range(kt)]

    def wob_copies():
        return [col_copy(wob_hbm, wob, j, 0, dm // 2, sem_late.at[3]) for j in range(kt)]

    def wa_copies(i):
        n = reg_per_iter * reg_rows
        r0 = _aligned(i * n, n)
        return [
            pltpu.make_async_copy(
                w.bitcast(I32).at[pl.ds(r0, n)],
                wa_flat.at[pl.ds((m * slots + 1) * reg_rows + r0, n)],
                sem_wa.at[i],
            )
            for m, w in enumerate((wq_hbm, wk_hbm, wv_hbm))
        ]

    def late_copies(i):
        r0 = pl.multiple_of(i * CHUNK, CHUNK)
        c0 = pl.multiple_of(i * LANES, LANES)
        return [
            pltpu.make_async_copy(
                woa_hbm.bitcast(I32).at[:, pl.ds(c0, LANES)], woa.at[i], sem_late.at[0]
            ),
            pltpu.make_async_copy(
                xa_hbm.at[pl.ds(r0, CHUNK)], xa.at[pl.ds(r0, CHUNK)], sem_late.at[1]
            ),
        ]

    def mem_copy():
        return pltpu.make_async_copy(mem_hbm, mem0, sem_late.at[2])

    def outb_copy(i):
        r0 = _aligned(i * CHUNK, CHUNK)
        return pltpu.make_async_copy(
            outb.at[pl.ds(r0, CHUNK)], out_hbm.at[pl.ds(r0, CHUNK), pl.ds(dm, dm)], sem_out.at[0]
        )

    def outa_copy(t):
        r0 = pl.multiple_of(t * seg, seg)
        return pltpu.make_async_copy(
            outa.at[pl.ds(r0, seg)], out_hbm.at[pl.ds(r0, seg), pl.ds(0, dm)], sem_out.at[1]
        )

    blk = (lax.broadcasted_iota(I32, (8, LANES), 1) >> 2) & 7

    def skew(x):
        x = [x[a] if a == 0 else pltpu.roll(x[a], 4 * a, 1) for a in range(kt)]
        return [x[-a % kt] for a in range(kt)]

    def unskew(x):
        for s in (1, 2, 4):
            take = (blk & s) != 0
            x = [jnp.where(take, x[(a - s) % kt], x[a]) for a in range(kt)]
        return [x[t] if t == 0 else pltpu.roll(x[t], LANES - 4 * t, 1) for t in range(kt)]

    def permute_wb(matrices, r0, n):
        items = [(m, _aligned(r0 + r, 8)) for r in range(0, n, 8) for m in matrices]
        live = {}
        for j in range(len(items) + PERM_LAG):
            if j < len(items):
                m, r = items[j]
                live[j] = skew([wb_raw[m * kt + a, pl.ds(r, 8), :] for a in range(kt)])
            if j >= PERM_LAG:
                m, r = items[j - PERM_LAG]
                for t, y in enumerate(unskew(live.pop(j - PERM_LAG))):
                    wb[m * kt + t, pl.ds(r, 8), :] = y

    def xb_rows(row0, n):
        w0 = _aligned(row0 // 2, n // 2)
        return jnp.concatenate(
            [_as_bf16(xb[j, pl.ds(w0, n // 2), :]) for j in range(kt)], axis=1
        )

    def q_project(i):
        row0 = pl.multiple_of(i * CHUNK, CHUNK)
        for t in range(kt):
            q_all[t, pl.ds(row0, CHUNK), :] = jnp.dot(
                xb_rows(row0, CHUNK), _as_bf16(wb[t]), preferred_element_type=F32
            )

    _start(wq_copies(0))
    _start(xb_copies(0))
    for u in range(1, WQ_BLOCKS):
        _start(wq_copies(u))
    for u in range(WQ_BLOCKS):
        _wait(wq_copies(u))
        if u == 0:
            _start(xb_copies(1))
        if u == WQ_BLOCKS - 1:
            _start(wkv_copies())
        permute_wb((0,), u * wq_rows, wq_rows)
    mem_copy().start()
    zero[...] = jnp.zeros((GRP, LANES), I32)
    k1[:, SUB:SUB + HALO, :] = jnp.zeros((kt, HALO, LANES), F32)
    v1[:, SUB:SUB + HALO, :] = jnp.zeros((kt, HALO, LANES), F32)
    _wait(xb_copies(0))

    half_iter = n_iter // 2

    def q_step_early(i, carry):
        @pl.when(i == 1)
        def _():
            _wait(xb_copies(1))
            _start(xb_copies(2))

        q_project(i)
        return carry

    def q_step_late(i, carry):
        q_project(i)
        n = dm // 2 // half_iter
        permute_wb((1, 2), (i - half_iter) * n, n)
        return carry

    lax.fori_loop(0, half_iter, q_step_early, None)
    _wait(wkv_copies())
    _wait(xb_copies(2))
    _start(wob_copies())
    _start(wa_copies(0))
    lax.fori_loop(half_iter, n_iter, q_step_late, None)
    _wait(wob_copies())

    b_scale = float((dm // B_HEADS) ** -0.5)
    lane_g = lax.broadcasted_iota(I32, (GRP, LANES), 1)
    row_g = lax.broadcasted_iota(I32, (GRP, LANES), 0)
    even1 = (lane_g & 1) == 0
    even2 = (lane_g & 2) == 0
    n_grp = SUB // GRP

    def gated(x, gate):
        return pltpu.bitcast(pltpu.bitcast(x, I32) | gate, F32)

    def b_project(row0, k_s, v_s):
        def tile(m, t, dst):
            y = jnp.dot(xb_rows(row0, SUB), _as_bf16(wb[m * kt + t]), preferred_element_type=F32)
            dst[t, HALO:HALO + SUB, :] = y
            return y

        return [
            functools.partial(tile, m, t, dst) for m, dst in ((1, k_s), (2, v_s)) for t in range(kt)
        ]

    def b_output(row0, o_s):
        def tile(n):
            o = jnp.concatenate([_as_bf16(o_s[t]) for t in range(kt)], axis=1)
            y = jnp.dot(o, _as_bf16(wob[n]), preferred_element_type=F32)
            outb[pl.ds(row0, SUB), n * LANES:(n + 1) * LANES] = y.astype(BF16)
            return y

        return [functools.partial(tile, n) for n in range(kt)]

    def b_weights(row0, k_s, p_s, may_mask):
        live = {}

        def products(g, gate):
            scale = gated(jnp.full((GRP, LANES), b_scale, F32), gate)
            rows = pl.ds(pl.multiple_of(row0 + g * GRP, GRP), GRP)
            q = [q_all[t, rows, :] * scale for t in range(kt)]
            out = []
            for w in range(B_WIN):
                acc = None
                for t in range(kt):
                    term = q[t] * k_s[t, pl.ds(HALO + g * GRP - B_DIL * w, GRP), :]
                    acc = term if acc is None else acc + term
                out.append((acc, pltpu.roll(acc, LANES - 1, 1), pltpu.roll(acc, 1, 1)))
            live[g] = out

        def pairs(g):
            out = [acc + jnp.where(even1, up, down) for acc, up, down in live[g]]
            live[g] = [(acc, pltpu.roll(acc, LANES - 2, 1), pltpu.roll(acc, 2, 1)) for acc in out]

        def softmax(g):
            logits = []
            for w, (acc, up, down) in enumerate(live.pop(g)):
                acc = acc + jnp.where(even2, up, down)
                if may_mask and g * GRP < B_DIL * w:
                    acc = jnp.where(row0 + g * GRP + row_g >= B_DIL * w, acc, NEG)
                logits.append(acc)
            top = functools.reduce(jnp.maximum, logits)
            e = [jnp.exp(x - top) for x in logits]
            for w in range(B_WIN):
                p_s[w, g * GRP:(g + 1) * GRP, :] = e[w]
            p_s[B_WIN, g * GRP:(g + 1) * GRP, :] = 1.0 / functools.reduce(jnp.add, e)

        def slot(j, gate):
            if 0 <= j - 2 < n_grp:
                softmax(j - 2)
            if 0 <= j - 1 < n_grp:
                pairs(j - 1)
            if j < n_grp:
                products(j, gate)

        return [functools.partial(slot, j) for j in range(n_grp + 2)]

    def b_mix(v_s, p_s, o_s):
        live = {}

        def slot(j, gate):
            if j >= 1:
                g = j - 1
                for a, words in enumerate(unskew(live.pop(g))):
                    o_s[a, g * GRP // 2:(g + 1) * GRP // 2, :] = words
            if j < n_grp:
                inv = gated(p_s[B_WIN, j * GRP:(j + 1) * GRP, :], gate)
                p = [p_s[w, j * GRP:(j + 1) * GRP, :] * inv for w in range(B_WIN)]
                o = []
                for t in range(kt):
                    acc = None
                    for w in range(B_WIN):
                        term = p[w] * v_s[t, pl.ds(HALO + j * GRP - B_DIL * w, GRP), :]
                        acc = term if acc is None else acc + term
                    o.append(pltpu.bitcast(acc.astype(BF16), I32))
                live[j] = skew(o)

        return [functools.partial(slot, j) for j in range(n_grp + 1)]

    def relayout_wa(slot):
        half = heads // 2
        per_d = half // 8
        for pair in range(8):
            for part in range(per_d):
                a = wa_reg[slot + 1, pl.ds(8 * ((2 * pair) * per_d + part), 8), :]
                b = wa_reg[slot + 1, pl.ds(8 * ((2 * pair + 1) * per_d + part), 8), :]
                lo = (a & 0xFFFF) | (b << 16)
                hi = lax.shift_right_logical(a, 16) | (b & -65536)
                wa_reg[slot, pl.ds(part * 64 + pair, 8, stride=8), :] = lo
                wa_reg[slot, pl.ds(half * 8 + part * 64 + pair, 8, stride=8), :] = hi

    def b_step(i, carry):
        @pl.when(i + 1 < n_iter)
        def _():
            _start(wa_copies(i + 1))

        @pl.when(i > 0)
        def _():
            outb_copy(i - 1).start()

        _start(late_copies(i))
        _wait(wa_copies(i))
        row_a = pl.multiple_of(i * CHUNK, CHUNK)
        row_b = pl.multiple_of(row_a + SUB, SUB)

        def pass_halo_k(gate):
            k1[:, 0:HALO, :] = k0[:, SUB:SUB + HALO, :]

        def pass_halo_v(gate):
            v_first = jnp.broadcast_to(v0[:, HALO:HALO + 1, :], (kt, HALO, LANES))
            v0[:, 0:HALO, :] = jnp.where(i == 0, v_first, v1[:, SUB:SUB + HALO, :])
            v1[:, 0:HALO, :] = v0[:, SUB:SUB + HALO, :]

        k0[:, 0:HALO, :] = k1[:, SUB:SUB + HALO, :]
        mxu = (
            b_project(row_a, k0, v0) + b_project(row_b, k1, v1)
            + b_output(row_a, ob0) + b_output(row_b, ob1)
        )
        shadow = [[] for _ in mxu]

        def place(jobs, first):
            for j, job in enumerate(jobs):
                shadow[first + j].append(job)

        place([pass_halo_k], kt - 1)
        place([pass_halo_v], 2 * kt - 1)
        place(b_weights(row_a, k0, p0, True), kt - 1)
        place(b_mix(v0, p0, ob0), 2 * kt - 1)
        place(b_weights(row_b, k1, p1, False), 3 * kt - 1)
        place(b_mix(v1, p1, ob1), 4 * kt - 1)
        for tile, jobs in zip(mxu, shadow):
            y = tile()
            if jobs:
                gate = pltpu.bitcast(y[SUB - GRP:SUB], I32) & zero[...]
            for job in jobs:
                job(gate)
        for m in range(3):
            for r in range(reg_per_iter):
                relayout_wa(m * slots + i * reg_per_iter + r)
        return carry

    lax.fori_loop(0, n_iter, b_step, None)
    outb_copy(n_iter - 1).start()

    pltpu.make_async_copy(woa, woa, sem_late.at[0]).wait()
    pltpu.make_async_copy(xa, xa, sem_late.at[1]).wait()
    mem_copy().wait()

    rows = n_mem + seg
    a_scale = float(LANES ** -0.5)
    hbuf[0:n_mem, :] = mem0[...].astype(F32)
    row = lax.broadcasted_iota(I32, (rows, rows), 0)
    col = lax.broadcasted_iota(I32, (rows, rows), 1)

    def a_step(t):
        r0 = pl.multiple_of(t * seg, seg)
        hbuf[n_mem:rows, :] = xa[pl.ds(r0, seg), :].astype(F32)
        visible = (row < n_mem) | (row >= col)
        qk, val = {}, {}

        def weight(m, h):
            entry = (h % 2) * (heads // 2) + h // 2
            return _as_bf16(wa[pl.ds(m * slots, regions), entry].reshape(dm // 2, LANES))

        def project_qk(h):
            w = jnp.concatenate([weight(0, h), weight(1, h)], axis=1)
            qk[h] = jnp.dot(hbuf[...], w, preferred_element_type=F32)

        def project_v(h):
            val[h] = jnp.dot(hbuf[...], weight(2, h), preferred_element_type=F32)

        def scores(h):
            y = qk.pop(h)
            k = y[:, LANES:].astype(BF16)
            s = lax.dot_general(
                y[:, :LANES], k, (((1,), (1,)), ((), ())), preferred_element_type=F32
            )
            s = jnp.where(visible, s * a_scale, NEG)
            e = jnp.exp(s - jnp.max(s, axis=1, keepdims=True))
            pbuf[h] = e / jnp.sum(e, axis=1, keepdims=True)

        def mix(h):
            obuf[:, h * LANES:(h + 1) * LANES] = jnp.dot(
                pbuf[h], val.pop(h).astype(BF16), preferred_element_type=F32
            )

        for j in range(2 * heads + LAG_P):
            if j < heads:
                project_qk(j)
            elif j < 2 * heads:
                project_v(j - heads)
            if 0 <= j - LAG_S < heads:
                scores(j - LAG_S)
            if 0 <= j - heads - LAG_P < heads:
                mix(j - heads - LAG_P)

        for n in range(kt):
            y = jnp.dot(obuf[...], _as_bf16(woa[n]), preferred_element_type=F32).astype(BF16)
            hbuf[0:n_mem, n * LANES:(n + 1) * LANES] = y[0:n_mem].astype(F32)
            outa[pl.ds(r0, seg), n * LANES:(n + 1) * LANES] = y[n_mem:rows]
        outa_copy(t).start()

    def a_steps(tt, carry):
        for u in range(A_UNROLL):
            a_step(tt * A_UNROLL + u)
        return carry

    lax.fori_loop(0, seq // seg // A_UNROLL, a_steps, None)

    pltpu.make_async_copy(outb, out_hbm.at[:, pl.ds(dm, dm)], sem_out.at[0]).wait()
    pltpu.make_async_copy(outa, out_hbm.at[:, pl.ds(0, dm)], sem_out.at[1]).wait()


@functools.partial(jax.jit, static_argnames=("A_seg_len",))
def pallas_concat_heads__memory_aug_recurrent_mem_tr__sliding_local_dilated__prompt_kernel(
    A_x: jax.Array,
    A_mem0: jax.Array,
    A_Wq: jax.Array,
    A_Wk: jax.Array,
    A_Wv: jax.Array,
    A_Wo: jax.Array,
    A_seg_len: int,
    B_x: jax.Array,
    B_wqkv: jax.Array,
    B_wo: jax.Array,
):
    batch, seq, dm = A_x.shape
    _, heads, dh = A_Wq.shape
    n_mem = A_mem0.shape[1]
    seg = int(A_seg_len)
    kt = dm // LANES
    rows = n_mem + seg
    n_iter = seq // CHUNK
    assert batch == 1 and B_x.shape == (1, seq, dm)
    assert dh == LANES and kt == 8 and dm // B_HEADS == 32 and heads % 16 == 0
    assert n_mem % 8 == 0 and seg % 16 == 0 and seq % (seg * A_UNROLL) == 0
    assert seq % CHUNK == 0 and n_iter == kt

    any_spec = pl.BlockSpec(memory_space=pl.ANY)
    scratch = [
        pltpu.VMEM((3 * (dm // 16 + 1), heads, 8, LANES), I32),
        pltpu.VMEM((kt, heads * dh // 2, LANES), I32),
        pltpu.VMEM((seq, dm), BF16),
        pltpu.VMEM((n_mem, dm), BF16),
        pltpu.VMEM((seq, dm), BF16),
        pltpu.VMEM((rows, dm), F32),
        pltpu.VMEM((rows, heads * dh), F32),
        pltpu.VMEM((heads, rows, rows), F32),
        pltpu.VMEM((kt, seq // 2, LANES), I32),
        pltpu.VMEM((3 * kt, dm // 2, LANES), I32),
        pltpu.VMEM((3 * kt, dm // 2, LANES), I32),
        pltpu.VMEM((kt, dm // 2, LANES), I32),
        pltpu.VMEM((seq, dm), BF16),
        pltpu.VMEM((kt, seq, LANES), F32),
        pltpu.VMEM((kt, HALO + SUB, LANES), F32),
        pltpu.VMEM((kt, HALO + SUB, LANES), F32),
        pltpu.VMEM((kt, HALO + SUB, LANES), F32),
        pltpu.VMEM((kt, HALO + SUB, LANES), F32),
        pltpu.VMEM((B_WIN + 1, SUB, LANES), F32),
        pltpu.VMEM((B_WIN + 1, SUB, LANES), F32),
        pltpu.VMEM((kt, SUB // 2, LANES), I32),
        pltpu.VMEM((kt, SUB // 2, LANES), I32),
        pltpu.VMEM((GRP, LANES), I32),
        pltpu.SemaphoreType.DMA((3,)),
        pltpu.SemaphoreType.DMA((WQ_BLOCKS + 1,)),
        pltpu.SemaphoreType.DMA((n_iter,)),
        pltpu.SemaphoreType.DMA((4,)),
        pltpu.SemaphoreType.DMA((2,)),
    ]
    out = pl.pallas_call(
        functools.partial(_kernel, seq=seq, dm=dm, heads=heads, n_mem=n_mem, seg=seg),
        out_shape=jax.ShapeDtypeStruct((seq, 2 * dm), BF16),
        in_specs=[any_spec] * 9,
        out_specs=any_spec,
        scratch_shapes=scratch,
        compiler_params=pltpu.CompilerParams(vmem_limit_bytes=100 * 1024 * 1024),
    )(
        A_x.reshape(seq, dm),
        A_mem0.reshape(n_mem, dm),
        A_Wq.reshape(dm * heads, dh),
        A_Wk.reshape(dm * heads, dh),
        A_Wv.reshape(dm * heads, dh),
        A_Wo.reshape(heads * dh, dm),
        B_x.reshape(seq, dm),
        B_wqkv,
        B_wo,
    )
    return out.reshape(1, seq, 2 * dm)
```

```python
import functools

import jax
import jax.numpy as jnp
from jax import lax
from jax.experimental import pallas as pl
from jax.experimental.pallas import tpu as pltpu

F32 = jnp.float32
BF16 = jnp.bfloat16
I32 = jnp.int32

LANES = 128
NEG = -1000000000.0

B_HEADS = 32
B_WIN = 8
B_DIL = 2

HALO = 16
SUB = 128
CHUNK = 2 * SUB
GRP = 16
WQ_BLOCKS = 4
PITCH = 516
PERM_LAG = 4
LAG_S = 4
LAG_P = 28
A_UNROLL = 4


def _as_bf16(words):
    return pltpu.bitcast(words, BF16)


def _start(copies):
    for cp in copies:
        cp.start()


def _wait(copies):
    for cp in copies:
        cp.wait()


def _aligned(start, multiple):
    return start if isinstance(start, int) else pl.multiple_of(start, multiple)


def _kernel(
    xa_hbm, mem_hbm, wq_hbm, wk_hbm, wv_hbm, woa_hbm, xb_hbm, wb_hbm, wob_hbm,
    out_hbm,
    wa_raw, wa, woa, xa, mem0, outa, hbuf, obuf, pbuf,
    xb, wb_raw, wb, wob, outb, q_all, k0, k1, v0, v1, p0, p1, ob0, ob1, zero,
    sem_xb, sem_wb, sem_wa, sem_late, sem_out,
    *, seq, dm, heads, n_mem, seg,
):
    kt = dm // LANES
    n_iter = seq // CHUNK
    regions = dm // 16
    reg_per_iter = regions // n_iter
    reg_rows = 16 * heads // 2
    chunk_rows = reg_per_iter * reg_rows

    def col_copy(src_hbm, dst, j, r0, n, sem):
        return pltpu.make_async_copy(
            src_hbm.bitcast(I32).at[pl.ds(r0, n), pl.ds(j * LANES, LANES)],
            dst.at[j, pl.ds(r0, n)],
            sem,
        )

    wq_rows = dm // 2 // WQ_BLOCKS
    xb_bounds = (0, CHUNK // 2, seq // 4, seq // 2)

    def wq_copies(u):
        return [col_copy(wb_hbm, wb_raw, j, u * wq_rows, wq_rows, sem_wb.at[u]) for j in range(kt)]

    def wkv_copies():
        return [
            col_copy(wb_hbm, wb_raw, j, 0, dm // 2, sem_wb.at[WQ_BLOCKS]) for j in range(kt, 3 * kt)
        ]

    def xb_copies(u):
        r0, r1 = xb_bounds[u:u + 2]
        return [col_copy(xb_hbm, xb, j, r0, r1 - r0, sem_xb.at[u]) for j in range(kt)]

    def wob_copies():
        return [col_copy(wob_hbm, wob, j, 0, dm // 2, sem_late.at[3]) for j in range(kt)]

    def wa_copies(i):
        r0 = _aligned(i * chunk_rows, chunk_rows)
        return [
            pltpu.make_async_copy(
                w.bitcast(I32).at[pl.ds(r0, chunk_rows)], wa_raw.at[i % 2, m], sem_wa.at[i]
            )
            for m, w in enumerate((wq_hbm, wk_hbm, wv_hbm))
        ]

    def late_copies(i):
        r0 = _aligned(i * CHUNK, CHUNK)
        c0 = _aligned(i * LANES, LANES)
        return [
            pltpu.make_async_copy(
                woa_hbm.bitcast(I32).at[:, pl.ds(c0, LANES)], woa.at[i], sem_late.at[0]
            ),
            pltpu.make_async_copy(
                xa_hbm.at[pl.ds(r0, CHUNK)], xa.at[pl.ds(r0, CHUNK)], sem_late.at[1]
            ),
        ]

    def mem_copy():
        return pltpu.make_async_copy(mem_hbm, mem0, sem_late.at[2])

    def outb_copy(i):
        r0 = _aligned(i * CHUNK, CHUNK)
        return pltpu.make_async_copy(
            outb.at[pl.ds(r0, CHUNK)], out_hbm.at[pl.ds(r0, CHUNK), pl.ds(dm, dm)], sem_out.at[0]
        )

    def outa_copy(t):
        r0 = pl.multiple_of(t * seg, seg)
        return pltpu.make_async_copy(
            outa.at[pl.ds(r0, seg)], out_hbm.at[pl.ds(r0, seg), pl.ds(0, dm)], sem_out.at[1]
        )

    blk = (lax.broadcasted_iota(I32, (8, LANES), 1) >> 2) & 7

    def skew(x):
        x = [x[a] if a == 0 else pltpu.roll(x[a], 4 * a, 1) for a in range(kt)]
        return [x[-a % kt] for a in range(kt)]

    def unskew(x):
        for s in (1, 2, 4):
            take = (blk & s) != 0
            x = [jnp.where(take, x[(a - s) % kt], x[a]) for a in range(kt)]
        return [x[t] if t == 0 else pltpu.roll(x[t], LANES - 4 * t, 1) for t in range(kt)]

    def permute_wb(matrices, r0, n):
        items = [(m, _aligned(r0 + r, 8)) for r in range(0, n, 8) for m in matrices]
        live = {}
        for j in range(len(items) + PERM_LAG):
            if j < len(items):
                m, r = items[j]
                live[j] = skew([wb_raw[m * kt + a, pl.ds(r, 8), :] for a in range(kt)])
            if j >= PERM_LAG:
                m, r = items[j - PERM_LAG]
                for t, y in enumerate(unskew(live.pop(j - PERM_LAG))):
                    wb[m * kt + t, pl.ds(r, 8), :] = y

    def xb_rows(row0, n):
        w0 = _aligned(row0 // 2, n // 2)
        return jnp.concatenate(
            [_as_bf16(xb[j, pl.ds(w0, n // 2), :]) for j in range(kt)], axis=1
        )

    def q_project(i):
        row0 = _aligned(i * CHUNK, CHUNK)
        for t in range(kt):
            q_all[t, pl.ds(row0, CHUNK), :] = jnp.dot(
                xb_rows(row0, CHUNK), _as_bf16(wb[t]), preferred_element_type=F32
            )

    _start(wq_copies(0))
    _start(xb_copies(0))
    for u in range(1, WQ_BLOCKS):
        _start(wq_copies(u))
    for u in range(WQ_BLOCKS):
        _wait(wq_copies(u))
        if u == 0:
            _start(xb_copies(1))
        if u == WQ_BLOCKS - 1:
            _start(wkv_copies())
        permute_wb((0,), u * wq_rows, wq_rows)
    mem_copy().start()
    zero[...] = jnp.zeros((GRP, LANES), I32)
    k1[:, SUB:SUB + HALO, :] = jnp.zeros((kt, HALO, LANES), F32)
    v1[:, SUB:SUB + HALO, :] = jnp.zeros((kt, HALO, LANES), F32)
    _wait(xb_copies(0))

    half_iter = n_iter // 2

    def q_step_early(i, carry):
        @pl.when(i == 1)
        def _():
            _wait(xb_copies(1))
            _start(xb_copies(2))

        q_project(i)
        return carry

    def q_step_late(i, carry):
        q_project(i)
        n = dm // 2 // half_iter
        permute_wb((1, 2), (i - half_iter) * n, n)
        return carry

    lax.fori_loop(0, half_iter, q_step_early, None)
    _wait(wkv_copies())
    _wait(xb_copies(2))
    _start(wob_copies())
    _start(wa_copies(0))
    _start(late_copies(0))
    lax.fori_loop(half_iter, n_iter, q_step_late, None)
    _wait(wob_copies())

    b_scale = float((dm // B_HEADS) ** -0.5)
    lane_g = lax.broadcasted_iota(I32, (GRP, LANES), 1)
    row_g = lax.broadcasted_iota(I32, (GRP, LANES), 0)
    even1 = (lane_g & 1) == 0
    even2 = (lane_g & 2) == 0
    n_grp = SUB // GRP

    def gated(x, gate):
        return pltpu.bitcast(pltpu.bitcast(x, I32) | gate, F32)

    def b_project(row0, k_s, v_s):
        def tile(m, t, dst):
            y = jnp.dot(xb_rows(row0, SUB), _as_bf16(wb[m * kt + t]), preferred_element_type=F32)
            dst[t, HALO:HALO + SUB, :] = y
            return y

        return [
            functools.partial(tile, m, t, dst) for m, dst in ((1, k_s), (2, v_s)) for t in range(kt)
        ]

    def b_output(row0, o_s):
        def tile(n):
            o = jnp.concatenate([_as_bf16(o_s[t]) for t in range(kt)], axis=1)
            y = jnp.dot(o, _as_bf16(wob[n]), preferred_element_type=F32)
            outb[pl.ds(row0, SUB), n * LANES:(n + 1) * LANES] = y.astype(BF16)
            return y

        return [functools.partial(tile, n) for n in range(kt)]

    def b_weights(row0, k_s, p_s, may_mask):
        live = {}

        def products(g, gate):
            scale = gated(jnp.full((GRP, LANES), b_scale, F32), gate)
            rows = pl.ds(pl.multiple_of(row0 + g * GRP, GRP), GRP)
            q = [q_all[t, rows, :] * scale for t in range(kt)]
            out = []
            for w in range(B_WIN):
                acc = None
                for t in range(kt):
                    term = q[t] * k_s[t, pl.ds(HALO + g * GRP - B_DIL * w, GRP), :]
                    acc = term if acc is None else acc + term
                out.append((acc, pltpu.roll(acc, LANES - 1, 1), pltpu.roll(acc, 1, 1)))
            live[g] = out

        def pairs(g):
            out = [acc + jnp.where(even1, up, down) for acc, up, down in live[g]]
            live[g] = [(acc, pltpu.roll(acc, LANES - 2, 1), pltpu.roll(acc, 2, 1)) for acc in out]

        def softmax(g):
            logits = []
            for w, (acc, up, down) in enumerate(live.pop(g)):
                acc = acc + jnp.where(even2, up, down)
                if may_mask and g * GRP < B_DIL * w:
                    acc = jnp.where(row0 + g * GRP + row_g >= B_DIL * w, acc, NEG)
                logits.append(acc)
            top = functools.reduce(jnp.maximum, logits)
            e = [jnp.exp(x - top) for x in logits]
            for w in range(B_WIN):
                p_s[w, g * GRP:(g + 1) * GRP, :] = e[w]
            p_s[B_WIN, g * GRP:(g + 1) * GRP, :] = 1.0 / functools.reduce(jnp.add, e)

        def slot(j, gate):
            if 0 <= j - 2 < n_grp:
                softmax(j - 2)
            if 0 <= j - 1 < n_grp:
                pairs(j - 1)
            if j < n_grp:
                products(j, gate)

        return [functools.partial(slot, j) for j in range(n_grp + 2)]

    def b_mix(v_s, p_s, o_s):
        live = {}

        def slot(j, gate):
            if j >= 1:
                g = j - 1
                for a, words in enumerate(unskew(live.pop(g))):
                    o_s[a, g * GRP // 2:(g + 1) * GRP // 2, :] = words
            if j < n_grp:
                inv = gated(p_s[B_WIN, j * GRP:(j + 1) * GRP, :], gate)
                p = [p_s[w, j * GRP:(j + 1) * GRP, :] * inv for w in range(B_WIN)]
                o = []
                for t in range(kt):
                    acc = None
                    for w in range(B_WIN):
                        term = p[w] * v_s[t, pl.ds(HALO + j * GRP - B_DIL * w, GRP), :]
                        acc = term if acc is None else acc + term
                    o.append(pltpu.bitcast(acc.astype(BF16), I32))
                live[j] = skew(o)

        return [functools.partial(slot, j) for j in range(n_grp + 1)]

    def relayout_wa(i, m, r, gate):
        half = heads // 2
        low, high = gate[0:8] | 0xFFFF, gate[0:8] | -65536
        for pair in range(8):
            for j in range(0, half, 8):
                src = r * reg_rows + 2 * pair * half + j
                a = wa_raw[i % 2, m, pl.ds(src, 8), :]
                b = wa_raw[i % 2, m, pl.ds(src + half, 8), :]
                dst = (m * heads + j) * PITCH + (i * reg_per_iter + r) * 8 + pair
                wa[pl.ds(dst, 8, stride=PITCH), :] = (a & low) | (b << 16)
                wa[pl.ds(dst + half * PITCH, 8, stride=PITCH), :] = (
                    lax.shift_right_logical(a, 16) | (b & high)
                )

    def b_step(i, carry):
        _wait(wa_copies(i))
        row_a = pl.multiple_of(i * CHUNK, CHUNK)
        row_b = pl.multiple_of(row_a + SUB, SUB)

        def start_copies(gate):
            @pl.when(i + 1 < n_iter)
            def _():
                _start(late_copies(i + 1))
                _start(wa_copies(i + 1))

            @pl.when(i > 0)
            def _():
                outb_copy(i - 1).start()

        def pass_halo_k(gate):
            k1[:, 0:HALO, :] = k0[:, SUB:SUB + HALO, :]

        def pass_halo_v(gate):
            v_first = jnp.broadcast_to(v0[:, HALO:HALO + 1, :], (kt, HALO, LANES))
            v0[:, 0:HALO, :] = jnp.where(i == 0, v_first, v1[:, SUB:SUB + HALO, :])
            v1[:, 0:HALO, :] = v0[:, SUB:SUB + HALO, :]

        k0[:, 0:HALO, :] = k1[:, SUB:SUB + HALO, :]
        mxu = (
            b_project(row_a, k0, v0) + b_project(row_b, k1, v1)
            + b_output(row_a, ob0) + b_output(row_b, ob1)
        )
        shadow = [[] for _ in mxu]

        def place(jobs, first):
            for j, job in enumerate(jobs):
                shadow[first + j].append(job)

        place([start_copies], 0)
        place([pass_halo_k], kt - 1)
        place([pass_halo_v], 2 * kt - 1)
        place(b_weights(row_a, k0, p0, True), kt - 1)
        place(b_mix(v0, p0, ob0), 2 * kt - 1)
        place(b_weights(row_b, k1, p1, False), 3 * kt - 1)
        place(b_mix(v1, p1, ob1), 4 * kt - 1)
        relayouts = [
            functools.partial(relayout_wa, i, m, r) for m in range(3) for r in range(reg_per_iter)
        ]
        place(relayouts[:7], 0)
        place(relayouts[7:17], 2 * kt)
        place(relayouts[17:], 5 * kt)
        for tile, jobs in zip(mxu, shadow):
            y = tile()
            if jobs:
                gate = pltpu.bitcast(y[0:GRP], I32) & zero[...]
            for job in jobs:
                job(gate)
        return carry

    lax.fori_loop(0, n_iter, b_step, None)
    outb_copy(n_iter - 1).start()

    pltpu.make_async_copy(woa, woa, sem_late.at[0]).wait()
    pltpu.make_async_copy(xa, xa, sem_late.at[1]).wait()
    mem_copy().wait()

    rows = n_mem + seg
    a_scale = float(LANES ** -0.5)
    hbuf[0:n_mem, :] = mem0[...].astype(F32)
    hbuf[n_mem:rows, :] = xa[0:seg, :].astype(F32)
    row = lax.broadcasted_iota(I32, (rows, rows), 0)
    col = lax.broadcasted_iota(I32, (rows, rows), 1)

    def a_step(t):
        r0 = pl.multiple_of(t * seg, seg)
        visible = (row < n_mem) | (row >= col)
        qk, val = {}, {}

        def weight(m, h):
            entry = (h % 2) * (heads // 2) + h // 2
            return _as_bf16(wa[pl.ds((m * heads + entry) * PITCH, dm // 2), :])

        def project_qk(h):
            w = jnp.concatenate([weight(0, h), weight(1, h)], axis=1)
            qk[h] = jnp.dot(hbuf[...], w, preferred_element_type=F32)

        def project_v(h):
            val[h] = jnp.dot(hbuf[...], weight(2, h), preferred_element_type=F32)

        def scores(h):
            y = qk.pop(h)
            k = y[:, LANES:].astype(BF16)
            s = lax.dot_general(
                y[:, :LANES], k, (((1,), (1,)), ((), ())), preferred_element_type=F32
            )
            s = jnp.where(visible, s * a_scale, NEG)
            e = jnp.exp(s - jnp.max(s, axis=1, keepdims=True))
            pbuf[h] = e / jnp.sum(e, axis=1, keepdims=True)

        def mix(h):
            obuf[:, h * LANES:(h + 1) * LANES] = jnp.dot(
                pbuf[h], val.pop(h).astype(BF16), preferred_element_type=F32
            )

        for j in range(2 * heads + LAG_P):
            if j < heads:
                project_qk(j)
            elif j < 2 * heads:
                project_v(j - heads)
            if 0 <= j - LAG_S < heads:
                scores(j - LAG_S)
            if 0 <= j - heads - LAG_P < heads:
                mix(j - heads - LAG_P)

        nxt = pl.multiple_of(jnp.minimum(r0 + seg, seq - seg), seg)
        hbuf[n_mem:rows, :] = xa[pl.ds(nxt, seg), :].astype(F32)
        for n in range(kt):
            y = jnp.dot(obuf[...], _as_bf16(woa[n]), preferred_element_type=F32).astype(BF16)
            hbuf[0:n_mem, n * LANES:(n + 1) * LANES] = y[0:n_mem].astype(F32)
            outa[pl.ds(r0, seg), n * LANES:(n + 1) * LANES] = y[n_mem:rows]
        outa_copy(t).start()

    def a_steps(tt, carry):
        for u in range(A_UNROLL):
            a_step(tt * A_UNROLL + u)
        return carry

    lax.fori_loop(0, seq // seg // A_UNROLL, a_steps, None)

    pltpu.make_async_copy(outb, out_hbm.at[:, pl.ds(dm, dm)], sem_out.at[0]).wait()
    pltpu.make_async_copy(outa, out_hbm.at[:, pl.ds(0, dm)], sem_out.at[1]).wait()


@functools.partial(jax.jit, static_argnames=("A_seg_len",))
def pallas_concat_heads__memory_aug_recurrent_mem_tr__sliding_local_dilated__prompt_kernel(
    A_x: jax.Array,
    A_mem0: jax.Array,
    A_Wq: jax.Array,
    A_Wk: jax.Array,
    A_Wv: jax.Array,
    A_Wo: jax.Array,
    A_seg_len: int,
    B_x: jax.Array,
    B_wqkv: jax.Array,
    B_wo: jax.Array,
):
    batch, seq, dm = A_x.shape
    _, heads, dh = A_Wq.shape
    n_mem = A_mem0.shape[1]
    seg = int(A_seg_len)
    kt = dm // LANES
    rows = n_mem + seg
    n_iter = seq // CHUNK
    assert batch == 1 and B_x.shape == (1, seq, dm)
    assert dh == LANES and kt == 8 and dm // B_HEADS == 32 and heads % 16 == 0
    assert n_mem % 8 == 0 and seg % 16 == 0 and seq % (seg * A_UNROLL) == 0
    assert seq % CHUNK == 0 and n_iter == kt

    any_spec = pl.BlockSpec(memory_space=pl.ANY)
    scratch = [
        pltpu.VMEM((2, 3, dm * heads // 2 // n_iter, LANES), I32),
        pltpu.VMEM((3 * heads * PITCH + 544, LANES), I32),
        pltpu.VMEM((kt, heads * dh // 2, LANES), I32),
        pltpu.VMEM((seq, dm), BF16),
        pltpu.VMEM((n_mem, dm), BF16),
        pltpu.VMEM((seq, dm), BF16),
        pltpu.VMEM((rows, dm), F32),
        pltpu.VMEM((rows, heads * dh), F32),
        pltpu.VMEM((heads, rows, rows), F32),
        pltpu.VMEM((kt, seq // 2, LANES), I32),
        pltpu.VMEM((3 * kt, dm // 2, LANES), I32),
        pltpu.VMEM((3 * kt, dm // 2, LANES), I32),
        pltpu.VMEM((kt, dm // 2, LANES), I32),
        pltpu.VMEM((seq, dm), BF16),
        pltpu.VMEM((kt, seq, LANES), F32),
        pltpu.VMEM((kt, HALO + SUB, LANES), F32),
        pltpu.VMEM((kt, HALO + SUB, LANES), F32),
        pltpu.VMEM((kt, HALO + SUB, LANES), F32),
        pltpu.VMEM((kt, HALO + SUB, LANES), F32),
        pltpu.VMEM((B_WIN + 1, SUB, LANES), F32),
        pltpu.VMEM((B_WIN + 1, SUB, LANES), F32),
        pltpu.VMEM((kt, SUB // 2, LANES), I32),
        pltpu.VMEM((kt, SUB // 2, LANES), I32),
        pltpu.VMEM((GRP, LANES), I32),
        pltpu.SemaphoreType.DMA((3,)),
        pltpu.SemaphoreType.DMA((WQ_BLOCKS + 1,)),
        pltpu.SemaphoreType.DMA((n_iter,)),
        pltpu.SemaphoreType.DMA((4,)),
        pltpu.SemaphoreType.DMA((2,)),
    ]
    out = pl.pallas_call(
        functools.partial(_kernel, seq=seq, dm=dm, heads=heads, n_mem=n_mem, seg=seg),
        out_shape=jax.ShapeDtypeStruct((seq, 2 * dm), BF16),
        in_specs=[any_spec] * 9,
        out_specs=any_spec,
        scratch_shapes=scratch,
        compiler_params=pltpu.CompilerParams(vmem_limit_bytes=100 * 1024 * 1024),
    )(
        A_x.reshape(seq, dm),
        A_mem0.reshape(n_mem, dm),
        A_Wq.reshape(dm * heads, dh),
        A_Wk.reshape(dm * heads, dh),
        A_Wv.reshape(dm * heads, dh),
        A_Wo.reshape(heads * dh, dm),
        B_x.reshape(seq, dm),
        B_wqkv,
        B_wo,
    )
    return out.reshape(1, seq, 2 * dm)
```
